```python
import os as _os
_os.environ.setdefault("JAX_PLATFORMS", "cpu")
import jax
import jax.numpy as jnp

def _softmax(x, axis=-1):
    return jax.nn.softmax(x, axis=axis)
def _gelu(x):
    return jax.nn.gelu(x, approximate=True)
def _silu(x):
    return jax.nn.silu(x)
def _sigmoid(x):
    return jax.nn.sigmoid(x)
def _layernorm(x, axis=-1, eps=1e-5):
    m = jnp.mean(x, axis=axis, keepdims=True)
    v = jnp.var(x, axis=axis, keepdims=True)
    return (x - m) / jnp.sqrt(v + eps)
def _scatter_add(tgt, idx, src, axis=0):
    return tgt.at[idx].add(src)
def _segment_sum(src, seg, n):
    return jax.ops.segment_sum(src, seg, n)
class _Rng:
    def __init__(self, key):
        self._k = key
    def _next(self):
        self._k, sub = jax.random.split(self._k)
        return sub
    def normal(self, shape):
        return jax.random.normal(self._next(), shape, dtype=jnp.bfloat16)
    def randint(self, lo, hi, shape):
        return jax.random.randint(self._next(), shape, lo, hi, dtype=jnp.int32)
    def uniform(self, shape, lo=0.0, hi=1.0):
        return jax.random.uniform(self._next(), shape, jnp.bfloat16, lo, hi)
    def permutation(self, n):
        return jax.random.permutation(self._next(), n)


kernel_name = 'concat_heads__ssm_conv_s4__grouped_kv_mqa__prompt'

def setup_inputs():
    _rng = _Rng(jax.random.key(int.from_bytes(__import__("os").urandom(4), "little")))
    _w = (lambda a: (lambda t: t.astype(jnp.bfloat16) if jnp.issubdtype(t.dtype, jnp.floating) else t)(jnp.asarray(a)))
    def _A_setup():
        B, L, D, N = 1, 2048, 448, 256
        A_re = -jnp.exp((lambda *s: _rng.normal(s) * 0.1)(D, N))
        A_im = jnp.pi * (lambda *s: _rng.normal(s) * 0.1)(D, N)
        B_re = (lambda *s: _rng.normal(s) * 0.1)(D, N)
        B_im = (lambda *s: _rng.normal(s) * 0.1)(D, N)
        C_re = (lambda *s: _rng.normal(s) * 0.1)(D, N)
        C_im = (lambda *s: _rng.normal(s) * 0.1)(D, N)
        log_dt = (lambda *s: _rng.normal(s) * 0.1)(D) * 0.5 - 4.0
        Dskip = (lambda *s: _rng.normal(s) * 0.05)(D)
        return {
            "u": _w((lambda *s: _rng.normal(s) * 0.05)(B, L, D)),
            "A_re": _w(A_re),
            "A_im": _w(A_im),
            "B_re": _w(B_re),
            "B_im": _w(B_im),
            "C_re": _w(C_re),
            "C_im": _w(C_im),
            "log_dt": _w(log_dt),
            "Dskip": _w(Dskip),
        }
    _A_in = _A_setup()

    def _B_setup():
        B, S, D, H = 1, 2048, 448, 16
        Dh = D // H
        return {
            "x": _w((lambda *s: _rng.normal(s) * 0.05)(B, S, D)),
            "wq": _w((lambda *s: _rng.normal(s) * 0.8)(D, H * Dh)),
            "wk": _w((lambda *s: _rng.normal(s) * 0.8)(D, Dh)),
            "wv": _w((lambda *s: _rng.normal(s) * 0.05)(D, Dh)),
            "wo": _w((lambda *s: _rng.normal(s) * 0.05)(H * Dh, D)),
        }
    _B_in = _B_setup()

    return {
        "A_u": _A_in["u"],
        "A_A_re": _A_in["A_re"],
        "A_A_im": _A_in["A_im"],
        "A_B_re": _A_in["B_re"],
        "A_B_im": _A_in["B_im"],
        "A_C_re": _A_in["C_re"],
        "A_C_im": _A_in["C_im"],
        "A_log_dt": _A_in["log_dt"],
        "A_Dskip": _A_in["Dskip"],
        "B_x": _B_in["x"],
        "B_wq": _B_in["wq"],
        "B_wk": _B_in["wk"],
        "B_wv": _B_in["wv"],
        "B_wo": _B_in["wo"],
    }

def reference(A_u, A_A_re, A_A_im, A_B_re, A_B_im, A_C_re, A_C_im, A_log_dt, A_Dskip, B_x, B_wq, B_wk, B_wv, B_wo):
    def _A_ref(u, A_re, A_im, B_re, B_im, C_re, C_im, log_dt, Dskip):
        Bsz, L, D = u.shape
        dt = jnp.exp(log_dt)[:, None]
        A = A_re + 1j * A_im
        Bc = B_re + 1j * B_im
        Cc = C_re + 1j * C_im
        logdA = dt * A
        dB = dt * Bc
        l = (lambda x, dt: x.astype(dt))(jnp.arange(L), A_re.dtype)
        P = jnp.exp(logdA[:, :, None] * l[None, None, :])
        K = jnp.einsum("dn,dnl,dn->dl", Cc, P, dB).real
        L2 = 2 * L
        Kp = jnp.pad(K, ((0, 0), (0, L)))
        up = (lambda x, *d: x.transpose(*d))(u, 0, 2, 1)
        up = jnp.pad(up, ((0, 0), (0, 0), (0, L)))
        Kf = (lambda x, axes=(-2,-1): jnp.fft.rfft2(x.astype(jnp.float32), axes=axes))(Kp[:, None, :], axes=(-2, -1))
        Uf = (lambda x, axes=(-2,-1): jnp.fft.rfft2(x.astype(jnp.float32), axes=axes))(up[:, :, None, :], axes=(-2, -1))
        Yf = Uf * Kf[None, :, :, :]
        y = (lambda x, s, axes=(-2,-1): jnp.fft.irfft2(x, s=s, axes=axes).astype(jnp.bfloat16))(Yf, (1, L2), axes=(-2, -1))[:, :, 0, :L]
        y = (lambda x, *d: x.transpose(*d))(y, 0, 2, 1) + u * Dskip[None, None, :]
        return y

    def _B_ref(x, wq, wk, wv, wo):
        B, S, D = x.shape
        H = 16
        Dh = D // H
        q = (lambda x, *d: x.transpose(*d))((x @ wq).reshape(B, S, H, Dh), 0, 2, 1, 3)
        k = x @ wk
        v = x @ wv
        scores = jnp.einsum("bhqd,bkd->bhqk", q, k) * (Dh ** -0.5)
        p = _softmax(scores, axis=-1)
        o = jnp.einsum("bhqk,bkd->bhqd", p, v)
        return (lambda x, *d: x.transpose(*d))(o, 0, 2, 1, 3).reshape(B, S, H * Dh) @ wo

    a = _A_ref(A_u, A_A_re, A_A_im, A_B_re, A_B_im, A_C_re, A_C_im, A_log_dt, A_Dskip)
    b = _B_ref(B_x, B_wq, B_wk, B_wv, B_wo)
    return jnp.concatenate([a, b], axis=-1)
```

```python
import ml_dtypes
import numpy as np

import jax
import jax.numpy as jnp
from jax import lax
from jax.experimental import pallas as pl
from jax.experimental.pallas import tpu as pltpu

F32 = jnp.float32
BF16 = jnp.bfloat16

L = 2048
D = 448
N = 256
H = 16
DH = D // H
TQ = 512
CK = 128
T = 128
NB = L // T
GC = 16
NG = D // GC
NPAIR = H // 2
NIT = (L // TQ) * NPAIR
QSCALE = float(DH ** -0.5 * np.log2(np.e))


def _dft_constants():
    t = np.arange(T, dtype=np.float64)
    f = np.arange(T, dtype=np.float64)
    ang = np.pi * np.outer(t, 2.0 * f + 1.0) / (2 * T)
    fwd = np.concatenate([np.cos(ang), -np.sin(ang)], axis=1)
    inv = np.concatenate([np.cos(ang).T, -np.sin(ang).T], axis=0) / T
    lag = np.arange(L).astype(np.float32).astype(ml_dtypes.bfloat16).astype(np.int64)

    def folded(block, lane_of):
        g = np.zeros((T, 2 * T))
        for i in range(T):
            lane = lane_of(int(lag[block * T + i]) - block * T)
            if lane is not None:
                g[lane] += fwd[i]
        return g

    g1 = folded(0, lambda r: 16 * (r % 8) + r // 8)
    g2 = folded(2, lambda r: 16 * ((r % 8) // 2) + r // 8 if r < T else 64)
    g4 = folded(4, lambda r: 64 * ((r % 8) // 4) + r // 8)
    g8 = folded(8, lambda r: r // 8)
    mats = np.stack([fwd, g1, g2, g4, g8]).astype(ml_dtypes.bfloat16)
    return mats, inv.astype(ml_dtypes.bfloat16)


_FWD_MATS, _INV_MAT = _dft_constants()


def _cmul(a, b):
    return a[0] * b[0] - a[1] * b[1], a[0] * b[1] + a[1] * b[0]


def _csq(a):
    t = a[0] * a[1]
    return a[0] * a[0] - a[1] * a[1], t + t


def _ssm_group(c0, r):
    rows = pl.ds(c0, GC)
    lane = lax.broadcasted_iota(jnp.int32, (8, 128), 1)

    edge = [[None] * 3 for _ in range(GC // 8)]
    dt16 = r.dt[rows, :]
    par = [p[rows, :].astype(F32) for p in (r.a_re, r.a_im, r.b_re, r.b_im, r.c_re, r.c_im)]
    for o in range(GC // 8):
        dt = dt16[8 * o:8 * o + 8]
        for nt in range(N // 128):
            a_re, a_im, b_re, b_im, c_re, c_im = [
                p[8 * o:8 * o + 8, 128 * nt:128 * nt + 128] for p in par]
            mag = jnp.exp(dt * a_re)
            ang = dt * a_im
            pw = {1: (mag * jnp.cos(ang), mag * jnp.sin(ang))}
            yield
            e = 1
            while e < L:
                pw[2 * e] = _csq(pw[e])
                e *= 2
            w = _cmul((c_re, c_im), (dt * b_re, dt * b_im))

            def put(tab, k, val):
                tab[o, 2 * nt, 8 * k:8 * k + 8, :] = val[0]
                tab[o, 2 * nt + 1, 8 * k:8 * k + 8, :] = val[1]

            p24 = _cmul(pw[8], pw[16])
            right = [(jnp.ones_like(mag), jnp.zeros_like(mag)), pw[8], pw[16], p24, pw[32],
                     _cmul(pw[8], pw[32]), _cmul(pw[16], pw[32]), _cmul(p24, pw[32])]
            for k in range(8):
                put(r.tab_r, k, right[k])
            put(r.tab_s, 0, pw[64])
            left = [w, _cmul(w, pw[1])]
            left += [_cmul(v, pw[2]) for v in left]
            left += [_cmul(v, pw[4]) for v in left]
            w512 = _cmul(w, pw[512])
            w1024 = _cmul(w, pw[1024])
            left += [w512, _cmul(w512, pw[4]), w1024, _cmul(w1024, pw[512])]
            for k in range(12):
                put(r.tab_l, k, (left[k][0], -left[k][1]))
            ends = (w512[0], w1024[0], w[0] * pw[2048][0] - w[1] * pw[2048][1])
            for k in range(3):
                edge[o][k] = ends[k] if nt == 0 else edge[o][k] + ends[k]
            yield
    edge = [[jnp.sum(v, axis=1, keepdims=True) for v in eo] for eo in edge]

    for c in range(8):
        lhs, rhs = [], []
        for o in range(2):
            lhs.append(jnp.concatenate(
                [jnp.concatenate([r.tab_l[o, q, pl.ds(c, 8, stride=8), :],
                                  r.tab_l[o, q, pl.ds(64 + c, 8, stride=8), :]], axis=0)
                 for q in range(4)], axis=1))
            cols = []
            for nt in range(N // 128):
                cur = tuple(r.tab_r[o, 2 * nt + q, pl.ds(c, 8, stride=8), :] for q in range(2))
                step = tuple(jnp.broadcast_to(r.tab_s[o, 2 * nt + q, c:c + 1, :], (8, 128))
                             for q in range(2))
                seq = [cur]
                for _ in range(7):
                    cur = _cmul(cur, step)
                    seq.append(cur)
                cols += [jnp.concatenate([s[q] for s in seq], axis=0) for q in range(2)]
            rhs.append(jnp.concatenate(cols, axis=1))
        lhs = jnp.concatenate(lhs, axis=0).astype(BF16)
        rhs = jnp.concatenate(rhs, axis=0).astype(BF16)
        kk = lax.dot_general(lhs, rhs, (((1,), (1,)), ((), ())), preferred_element_type=F32)
        r.kd[16 * c:16 * c + 8, :] = jnp.where(lane < 64, kk[0:8], kk[16:24])
        r.kd[16 * c + 8:16 * c + 16, :] = jnp.where(lane < 64, kk[8:16], kk[24:32])
        yield

    x = [r.kd[pl.ds(a, 8, stride=16), :] for a in range(12)]

    def rolled(v, shift):
        shift %= 128
        return pltpu.roll(v, shift, 1) if shift else v

    def gather16(srcs, first):
        out = None
        for k, v in enumerate(srcs):
            piece = rolled(v, 16 * k - first)
            out = piece if out is None else jnp.where(lane < 16 * k, out, piece)
        return out

    near, mid2, mid4, far = [], [], [], []
    for m in range(2):
        near.append([gather16(x[0:8], 64 * o + 16 * m) for o in range(2)])
    yield
    for m in range(2):
        blk = []
        for o in range(2):
            top = rolled(x[0], 64 - (64 * o + 48)) if m == 0 else edge[o][0]
            blk.append(jnp.where(lane == 64, top, gather16(x[0:8:2], 64 * o + 32 + 16 * m)))
        mid2.append(blk)
    t4 = [jnp.where(lane < 64, rolled(x[8], -64 * o), rolled(x[9], 64 - 64 * o)) for o in range(2)]
    t8 = [jnp.where(lane < 64, rolled(x[10], -64 * o), rolled(x[11], 64 - 64 * o)) for o in range(2)]
    for m in range(4):
        blk = [rolled(t4[o], -16 * m) for o in range(2)]
        if m == 3:
            blk = [jnp.where(lane == 16, edge[o][1], blk[o]) for o in range(2)]
        mid4.append(blk)
    for m in range(8):
        blk = [rolled(t8[o], -16 * m) for o in range(2)]
        if m == 7:
            blk = [jnp.where(lane == 16, edge[o][2], blk[o]) for o in range(2)]
        far.append(blk)
    yield

    def stack(blocks):
        return jnp.concatenate([v for blk in blocks for v in blk], axis=0).astype(BF16)

    u = r.u[rows, :]
    lhs = jnp.concatenate([u[:, T * j:T * j + T] for j in range(NB)], axis=0)
    r.uf[...] = jnp.dot(lhs, r.fwd[0], preferred_element_type=F32)
    yield
    kf = jnp.concatenate(
        [jnp.dot(stack(b), r.fwd[i], preferred_element_type=F32)
         for i, b in ((1, near), (2, mid2), (3, mid4), (4, far))], axis=0)
    sign = jnp.where(lax.broadcasted_iota(jnp.int32, (GC, 128), 1) % 2 == 0, 1.0, -1.0)
    r.kf[0:GC, :] = kf[0:GC]
    for m in range(1, NB):
        cur, prev = kf[GC * m:GC * m + GC], kf[GC * m - GC:GC * m]
        r.kf[GC * m:GC * m + GC, 0:T] = cur[:, :T] - sign * prev[:, T:]
        r.kf[GC * m:GC * m + GC, T:] = cur[:, T:] + sign * prev[:, :T]
    yield

    IB = 4
    for o in range(GC // 8):
        def tile(ref, b):
            s = slice(GC * b + 8 * o, GC * b + 8 * o + 8)
            return ref[s, 0:T], ref[s, T:]
        for i0 in range(0, NB, IB):
            acc = [None] * IB
            for j in range(i0 + IB):
                uj = tile(r.uf, j)
                for i in range(max(i0, j), i0 + IB):
                    pr = _cmul(tile(r.kf, i - j), uj)
                    a = acc[i - i0]
                    acc[i - i0] = pr if a is None else (a[0] + pr[0], a[1] + pr[1])
            for i in range(i0, i0 + IB):
                s = slice(GC * i + 8 * o, GC * i + 8 * o + 8)
                r.yf[s, 0:T] = acc[i - i0][0]
                r.yf[s, T:] = acc[i - i0][1]
            yield

    y = jnp.dot(r.yf[...].astype(BF16), r.inv[...], preferred_element_type=F32)
    skip = r.dskip[rows, :]
    for i in range(NB):
        r.yt[rows, T * i:T * i + T] = (
            y[GC * i:GC * i + GC] + skip * r.u[rows, T * i:T * i + T].astype(F32))
    yield


class _Refs:
    pass


def _kernel(ut_hbm, are_hbm, aim_hbm, bre_hbm, bim_hbm, cre_hbm, cim_hbm, ldt_ref, dsk_ref,
            xt_hbm, wq_hbm, wkt_ref, wvt_ref, wo_hbm, fwd_hbm, inv_hbm,
            out_hbm,
            u_v, are_v, aim_v, bre_v, bim_v, cre_v, cim_v, x_v, wq_v, wo_v, fwd_v, inv_v,
            wkv_s, wqt_s, wot_s, ke_s, ko_s, ve_s, vo_s, q_s, sa_s, sb_s, ot_s,
            dt_s, dskip_s, tab_l, tab_r, tab_s, kd_s, uf_s, kf_s, yf_s, yt_s,
            stage_a, stage_b, in_sem, out_sem):
    r = _Refs()
    r.u, r.a_re, r.a_im, r.b_re, r.b_im, r.c_re, r.c_im = u_v, are_v, aim_v, bre_v, bim_v, cre_v, cim_v
    r.fwd, r.inv, r.dt, r.dskip = fwd_v, inv_v, dt_s, dskip_s
    r.tab_l, r.tab_r, r.tab_s, r.kd, r.uf, r.kf, r.yf, r.yt = (
        tab_l, tab_r, tab_s, kd_s, uf_s, kf_s, yf_s, yt_s)

    pairs = [(wq_hbm, wq_v), (xt_hbm, x_v), (are_hbm, are_v), (aim_hbm, aim_v), (bre_hbm, bre_v),
             (bim_hbm, bim_v), (cre_hbm, cre_v), (cim_hbm, cim_v), (ut_hbm, u_v),
             (fwd_hbm, fwd_v), (inv_hbm, inv_v), (wo_hbm, wo_v)]
    loads = [pltpu.make_async_copy(s, d, in_sem.at[i]) for i, (s, d) in enumerate(pairs)]
    for cp in loads:
        cp.start()

    def column(row):
        wide = jnp.concatenate([row, jnp.zeros((1, 512 - D), F32)], axis=1)
        return jnp.broadcast_to(wide, (128, 512)).T[:D]

    dt_s[...] = column(jnp.exp(ldt_ref[...].astype(F32)).astype(BF16).astype(F32))
    dskip_s[...] = column(dsk_ref[...].astype(F32))
    tab_l[:, :, 96:128, :] = jnp.zeros((GC // 8, 4, 32, 128), F32)
    wkv_s[...] = jnp.zeros(wkv_s.shape, F32)
    wkv_s[0:DH, :] = wkt_ref[...].astype(F32)
    wkv_s[32:32 + DH, :] = wvt_ref[...].astype(F32)

    def transposed(w_ref):
        w = w_ref[...].astype(F32)
        w = jnp.concatenate([w, jnp.zeros((D, 512 - D), F32)], axis=1)
        w = jnp.concatenate([w, jnp.zeros((512 - D, 512), F32)], axis=0)
        return w.T[:D, :D]

    loads[0].wait()
    wqt_s[0:D, :] = transposed(wq_v) * QSCALE
    wqt_s[D:, :] = jnp.zeros((8, D), F32)
    loads[1].wait()

    kv = jnp.dot(wkv_s[...].astype(BF16), x_v[...], preferred_element_type=F32)
    k_t = kv[0:32]
    v_t = jnp.where(lax.broadcasted_iota(jnp.int32, (32, L), 0) == DH, 1.0, kv[32:64])
    ve_s[...] = v_t.astype(BF16)
    vo_s[...] = pltpu.roll(v_t, 4, 0).astype(BF16)
    k_all = jnp.concatenate([k_t, pltpu.roll(k_t, 4, 0), jnp.zeros((64, L), F32)], axis=0).T
    ke_s[...] = k_all[:, 0:32].astype(BF16)
    ko_s[...] = k_all[:, 32:64].astype(BF16)

    def project_q(it):
        w = wqt_s[pl.ds(pl.multiple_of((it % NPAIR) * 2 * DH, 8), 64), :].astype(BF16)
        cols = pl.ds(pl.multiple_of((it // NPAIR) * TQ, TQ), TQ)
        return jnp.dot(w, x_v[:, cols], preferred_element_type=F32)

    def head_step(k_ref, q_t, dst, src, m_src, v_ref, side):
        m_new = acc = None
        for c in range(L // CK):
            ks = slice(c * CK, (c + 1) * CK)
            if dst is not None:
                s = jnp.dot(k_ref[ks, :], q_t, preferred_element_type=F32)
                dst[ks, :] = s
                mc = jnp.max(s.reshape(CK // 8, 8, TQ), axis=0)
                m_new = mc if m_new is None else jnp.maximum(m_new, mc)
            if src is not None:
                p = jnp.exp2(src[ks, :] - m_src).astype(BF16)
                o = jnp.dot(v_ref[:, ks], p, preferred_element_type=F32)
                acc = o if acc is None else acc + o
            side()
        if dst is not None:
            m_new = jnp.max(m_new, axis=0, keepdims=True)
        return m_new, acc

    def iteration(it, m_even, with_ssm, last=False):
        if with_ssm:
            work = _ssm_group(pl.multiple_of(((it + NG - 4) % NG) * GC, GC), r)
        else:
            work = iter(())
        side = lambda: next(work, None)
        q_odd = q_s[24:56, :].astype(BF16)
        if not last:
            q_next = project_q(it + 1)
            q_s[...] = q_next
        m_odd, acc_e = head_step(ko_s, q_odd, sb_s, sa_s, m_even, ve_s, side)
        if last:
            m_even, acc_o = head_step(None, None, None, sb_s, m_odd, vo_s, side)
        else:
            m_even, acc_o = head_step(ke_s, q_s[0:32, :].astype(BF16), sa_s, sb_s, m_odd, vo_s, side)
        for _ in work:
            pass
        o_e = acc_e * (1.0 / acc_e[DH:DH + 1])
        o_o = acc_o * (1.0 / acc_o[0:1])
        mixed = jnp.where(lax.broadcasted_iota(jnp.int32, (8, TQ), 0) < 4, o_e[24:32], o_o[0:8])
        base = pl.multiple_of((it % NPAIR) * 2 * DH, 8)
        ot_s[pl.ds(base, 2 * DH), :] = jnp.concatenate([o_e[0:24], mixed, o_o[8:32]], axis=0)
        return m_even

    def b_copy(j):
        return pltpu.make_async_copy(
            stage_b.at[j], out_hbm.at[pl.ds(j * TQ, TQ), pl.ds(384, 512)], out_sem.at[j])

    def a_copy(c):
        return pltpu.make_async_copy(
            stage_a.at[c], out_hbm.at[:, pl.ds(128 * c, 128)], out_sem.at[4 + c])

    def finish_tile(j):
        cols = pl.ds(pl.multiple_of(j * TQ, TQ), TQ)
        o = jnp.dot(wot_s[...], ot_s[...].astype(BF16), preferred_element_type=F32)
        z = jnp.concatenate([yt_s[384:D, cols], o], axis=0)
        stage_b[j] = z.T.astype(BF16)
        b_copy(j).start()

    def finish_channels(c):
        stage_a[c] = yt_s[pl.ds(pl.multiple_of(128 * c, 128), 128), :].T.astype(BF16)
        a_copy(c).start()

    q_s[...] = project_q(0)
    m, _ = head_step(ke_s, q_s[0:32, :].astype(BF16), sa_s, None, None, None, lambda: None)
    for cp in loads[2:]:
        cp.wait()
    wot_s[...] = transposed(wo_v).astype(BF16)

    def body(with_ssm):
        def run(it, m):
            m = iteration(it, m, with_ssm)

            @pl.when(it % NPAIR == NPAIR - 1)
            def _():
                finish_tile(it // NPAIR)

            if with_ssm:
                @pl.when(jnp.logical_and(it % NPAIR == 3, it > NPAIR))
                def _():
                    finish_channels(it // NPAIR - 1)
            return m
        return run

    m = lax.fori_loop(0, NG, body(True), m)
    m = lax.fori_loop(NG, NIT - 1, body(False), m)
    iteration(NIT - 1, m, False, last=True)
    finish_tile(L // TQ - 1)
    for j in range(L // TQ):
        b_copy(j).wait()
    for c in range(3):
        a_copy(c).wait()


@jax.jit
def pallas_concat_heads__ssm_conv_s4__grouped_kv_mqa__prompt_kernel(
    A_u: jax.Array,
    A_A_re: jax.Array,
    A_A_im: jax.Array,
    A_B_re: jax.Array,
    A_B_im: jax.Array,
    A_C_re: jax.Array,
    A_C_im: jax.Array,
    A_log_dt: jax.Array,
    A_Dskip: jax.Array,
    B_x: jax.Array,
    B_wq: jax.Array,
    B_wk: jax.Array,
    B_wv: jax.Array,
    B_wo: jax.Array,
):
    hbm = pl.BlockSpec(memory_space=pl.ANY)
    vmem = pl.BlockSpec(memory_space=pltpu.VMEM)
    scratch = [
        pltpu.VMEM((D, L), BF16),
        *[pltpu.VMEM((D, N), BF16) for _ in range(6)],
        pltpu.VMEM((D, L), BF16),
        pltpu.VMEM((D, D), BF16), pltpu.VMEM((D, D), BF16),
        pltpu.VMEM((5, T, 2 * T), BF16), pltpu.VMEM((2 * T, T), BF16),
        pltpu.VMEM((64, D), F32),
        pltpu.VMEM((D + 8, D), F32),
        pltpu.VMEM((D, D), BF16),
        pltpu.VMEM((L, 32), BF16), pltpu.VMEM((L, 32), BF16),
        pltpu.VMEM((32, L), BF16), pltpu.VMEM((32, L), BF16),
        pltpu.VMEM((64, TQ), F32),
        pltpu.VMEM((L, TQ), F32), pltpu.VMEM((L, TQ), F32),
        pltpu.VMEM((D, TQ), F32),
        pltpu.VMEM((D, 128), F32), pltpu.VMEM((D, 128), F32),
        pltpu.VMEM((GC // 8, 4, 128, 128), F32),
        pltpu.VMEM((GC // 8, 4, 64, 128), F32),
        pltpu.VMEM((GC // 8, 4, 8, 128), F32),
        pltpu.VMEM((128, 128), F32),
        pltpu.VMEM((NB * GC, 2 * T), F32), pltpu.VMEM((NB * GC, 2 * T), F32),
        pltpu.VMEM((NB * GC, 2 * T), F32),
        pltpu.VMEM((D, L), F32),
        pltpu.VMEM((3, L, 128), BF16), pltpu.VMEM((L // TQ, TQ, 512), BF16),
        pltpu.SemaphoreType.DMA((12,)), pltpu.SemaphoreType.DMA((7,)),
    ]
    out = pl.pallas_call(
        _kernel,
        out_shape=jax.ShapeDtypeStruct((L, 2 * D), BF16),
        in_specs=[hbm] * 7 + [vmem, vmem, hbm, hbm, vmem, vmem, hbm, hbm, hbm],
        out_specs=hbm,
        scratch_shapes=scratch,
        compiler_params=pltpu.CompilerParams(vmem_limit_bytes=100 * 1024 * 1024),
    )(A_u[0].T, A_A_re, A_A_im, A_B_re, A_B_im, A_C_re, A_C_im,
      A_log_dt.reshape(1, D), A_Dskip.reshape(1, D),
      B_x[0].T, B_wq, B_wk.T, B_wv.T, B_wo, _FWD_MATS, _INV_MAT)
    return out[None]
```

```python
import ml_dtypes
import numpy as np

import jax
import jax.numpy as jnp
from jax import lax
from jax.experimental import pallas as pl
from jax.experimental.pallas import tpu as pltpu

F32 = jnp.float32
BF16 = jnp.bfloat16

L = 2048
D = 448
N = 256
H = 16
DH = D // H
TQ = 512
CK = 128
T = 128
NB = L // T
GC = 16
NG = D // GC
NPAIR = H // 2
NIT = (L // TQ) * NPAIR

PLACEMENT = {
    'shift': {5: -0.6, 15: -0.2, 18: 0.6, 27: -0.8},
    'cut': {1: 96, 3: 64, 5: 96, 9: 48, 30: 64, 31: 64},
    'free': {},
    'turn': {},
    'matmuls': {6: 2, 17: 0},
}

QSCALE = float(DH ** -0.5 * np.log2(np.e))


def _dft_constants():
    t = np.arange(T, dtype=np.float64)
    f = np.arange(T, dtype=np.float64)
    ang = np.pi * np.outer(t, 2.0 * f + 1.0) / (2 * T)
    fwd = np.concatenate([np.cos(ang), -np.sin(ang)], axis=1)
    inv = np.concatenate([np.cos(ang).T, -np.sin(ang).T], axis=0) / T
    lag = np.arange(L).astype(np.float32).astype(ml_dtypes.bfloat16).astype(np.int64)

    def folded(block, lane_of):
        g = np.zeros((T, 2 * T))
        for i in range(T):
            lane = lane_of(int(lag[block * T + i]) - block * T)
            if lane is not None:
                g[lane] += fwd[i]
        return g

    g1 = folded(0, lambda r: 16 * (r % 8) + r // 8)
    g2 = folded(2, lambda r: 16 * ((r % 8) // 2) + r // 8 if r < T else 64)
    g4 = folded(4, lambda r: 64 * ((r % 8) // 4) + r // 8)
    g8 = folded(8, lambda r: r // 8)
    mats = np.stack([fwd, g1, g2, g4, g8]).astype(ml_dtypes.bfloat16)
    return mats, inv.astype(ml_dtypes.bfloat16)


_FWD_MATS, _INV_MAT = _dft_constants()


PITCH = 9


def _aligned(i, n):
    return i if isinstance(i, int) else pl.multiple_of(i, n)


def _cmul(a, b):
    return a[0] * b[0] - a[1] * b[1], a[0] * b[1] + a[1] * b[0]


def _cmul_conj(a, b):
    return a[0] * b[0] + a[1] * b[1], a[1] * b[0] - a[0] * b[1]


def _csq(a):
    t = a[0] * a[1]
    return a[0] * a[0] - a[1] * a[1], t + t


def _ssm_powers(c0, r):
    rows = pl.ds(c0, GC)
    edge = [[None] * 3 for _ in range(GC // 8)]
    for o in range(GC // 8):
        for nt in range(N // 128):
            def param(ref):
                return ref[rows, 128 * nt:128 * nt + 128].astype(F32)[8 * o:8 * o + 8]

            def put(tab, k, val):
                tab[o, 2 * nt, PITCH * k:PITCH * k + 8, :] = val[0]
                tab[o, 2 * nt + 1, PITCH * k:PITCH * k + 8, :] = val[1]

            dt = r.dt[rows, :][8 * o:8 * o + 8]
            mag = jnp.exp(dt * param(r.a_re))
            ang = dt * param(r.a_im)
            p1 = (mag * jnp.cos(ang), mag * jnp.sin(ang))
            yield 130, list(p1)
            w = _cmul((param(r.c_re), param(r.c_im)), (dt * param(r.b_re), dt * param(r.b_im)))
            w = (w[0], -w[1])
            put_left = lambda k, v: put(r.tab_l, k, v)
            put_left(0, w)
            cur = w
            for k in range(1, 8):
                cur = _cmul_conj(cur, p1)
                put_left(k, cur)
            p4 = _csq(_csq(p1))
            p8 = _csq(p4)
            yield 75, [*cur, *p8]
            put(r.tab_r, 0, (jnp.ones_like(mag), jnp.zeros_like(mag)))
            cur = p8
            for k in range(1, 8):
                put(r.tab_r, k, cur)
                cur = _cmul(cur, p8)
            put(r.tab_s, 0, cur)
            yield 45, list(cur)
            p512 = _csq(_csq(_csq(cur)))
            w512 = _cmul_conj(w, p512)
            put_left(8, w512)
            w516 = _cmul_conj(w512, p4)
            put_left(9, w516)
            w1024 = _cmul_conj(w512, p512)
            put_left(10, w1024)
            w1536 = _cmul_conj(w1024, p512)
            put_left(11, w1536)
            ends = (w512[0], w1024[0], w1536[0] * p512[0] + w1536[1] * p512[1])
            for k in range(3):
                edge[o][k] = ends[k] if nt == 0 else edge[o][k] + ends[k]
            yield 50, [*w516, edge[o][2]]
        for k in range(3):
            r.edge[o, k] = edge[o][k]


def _ssm_kernel_values(r):
    lane = lax.broadcasted_iota(jnp.int32, (8, 128), 1)
    for c in range(8):
        rhs = []
        for nt in range(N // 128):
            both = []
            for o in range(2):
                cur = tuple(r.tab_r[o, 2 * nt + q, pl.ds(c, 8, stride=PITCH), :] for q in range(2))
                step = tuple(jnp.broadcast_to(r.tab_s[o, 2 * nt + q, c:c + 1, :], (8, 128))
                             for q in range(2))
                seq = [cur]
                for _ in range(7):
                    cur = _cmul(cur, step)
                    seq.append(cur)
                both.append(jnp.concatenate(
                    [jnp.concatenate([v[q] for v in seq], axis=0) for q in range(2)],
                    axis=1).astype(BF16))
                yield 52, list(cur)
            rhs.append(jnp.concatenate(both, axis=0))

        def matmul(c=c, rhs=rhs):
            lhs = jnp.concatenate(
                [jnp.concatenate([r.tab_l[o, q, pl.ds(k + c, 8, stride=PITCH), :]
                                  for o in range(2) for k in (0, 8 * PITCH)], axis=0)
                 for q in range(4)], axis=1).astype(BF16)
            kk = lax.dot_general(lhs, jnp.concatenate(rhs, axis=1), (((1,), (1,)), ((), ())),
                                 preferred_element_type=F32)
            r.kd[17 * c:17 * c + 8, :] = jnp.where(lane < 64, kk[0:8], kk[16:24])
            r.kd[17 * c + 8:17 * c + 16, :] = jnp.where(lane < 64, kk[8:16], kk[24:32])

        r.mxu.append(matmul)
        yield 20, []


def _ssm_spectra(c0, r):
    rows = pl.ds(c0, GC)
    lane = lax.broadcasted_iota(jnp.int32, (8, 128), 1)
    edge = [[jnp.sum(r.edge[o, k], axis=1, keepdims=True) for k in range(3)] for o in range(2)]
    x = [r.kd[pl.ds(a, 8, stride=17), :] for a in range(12)]

    def rolled(v, shift):
        shift %= 128
        return pltpu.roll(v, shift, 1) if shift else v

    def gather16(srcs, first):
        out = None
        for k, v in enumerate(srcs):
            piece = rolled(v, 16 * k - first)
            out = piece if out is None else jnp.where(lane < 16 * k, out, piece)
        return out

    near, mid2, mid4, far = [], [], [], []
    for m in range(2):
        near.append([gather16(x[0:8], 64 * o + 16 * m) for o in range(2)])
    yield 100, [v for blk in near for v in blk]
    for m in range(2):
        blk = []
        for o in range(2):
            top = rolled(x[0], 64 - (64 * o + 48)) if m == 0 else edge[o][0]
            blk.append(jnp.where(lane == 64, top, gather16(x[0:8:2], 64 * o + 32 + 16 * m)))
        mid2.append(blk)
    t4 = [jnp.where(lane < 64, rolled(x[8], -64 * o), rolled(x[9], 64 - 64 * o)) for o in range(2)]
    t8 = [jnp.where(lane < 64, rolled(x[10], -64 * o), rolled(x[11], 64 - 64 * o)) for o in range(2)]
    for m in range(4):
        blk = [rolled(t4[o], -16 * m) for o in range(2)]
        if m == 3:
            blk = [jnp.where(lane == 16, edge[o][1], blk[o]) for o in range(2)]
        mid4.append(blk)
    for m in range(8):
        blk = [rolled(t8[o], -16 * m) for o in range(2)]
        if m == 7:
            blk = [jnp.where(lane == 16, edge[o][2], blk[o]) for o in range(2)]
        far.append(blk)
    yield 100, [v for blk in mid2 + mid4[3:] + far[7:] for v in blk]

    def stack(blocks):
        return jnp.concatenate([v for blk in blocks for v in blk], axis=0).astype(BF16)

    packed = [[(stack(near), 1), (stack(mid2), 2)], [(stack(mid4), 3)],
              [(stack(far[:4]), 4)], [(stack(far[4:]), 4)]]
    sign = jnp.where(lane % 2 == 0, 1.0, -1.0)
    sign = jnp.concatenate([sign] * (GC // 8), axis=0)
    above = []

    def transform(q):
        u = r.u[rows, 4 * T * q:4 * T * (q + 1)]
        lhs = jnp.concatenate([u[:, T * j:T * j + T] for j in range(4)], axis=0)
        spec = jnp.dot(lhs, r.fwd[0], preferred_element_type=F32)
        r.uf[4 * GC * q:4 * GC * (q + 1), :] = spec
        r.us[4 * GC * q:4 * GC * (q + 1), :] = spec[:, :T] + spec[:, T:]
        kf = jnp.concatenate(
            [jnp.dot(v, r.fwd[i], preferred_element_type=F32) for v, i in packed[q]], axis=0)
        blocks = [kf[GC * m:GC * m + GC] for m in range(4)] + above
        above[:] = blocks[:1]
        if q == 0:
            r.kf[0:GC, 0:T] = blocks[0][:, :T]
            r.kf[0:GC, T:] = blocks[0][:, :T] + blocks[0][:, T:]
            r.kd2[0:GC, :] = blocks[0][:, T:] - blocks[0][:, :T]
        anchors = []
        for m in range(1, len(blocks)):
            cur, prev = blocks[m], blocks[m - 1]
            k_re = cur[:, :T] - sign * prev[:, T:]
            k_im = cur[:, T:] + sign * prev[:, :T]
            at = slice(GC * (4 * q + m), GC * (4 * q + m + 1))
            r.kf[at, 0:T] = k_re
            r.kd2[at, :] = k_im - k_re
            k_im = k_re + k_im
            r.kf[at, T:] = k_im
            anchors = [k_re[8:], k_im[8:]]
        return anchors

    r.transform = transform


def _ssm_products(r):
    for i in reversed(range(NB)):
        for o in range(GC // 8):
            acc = None
            for j in range(i + 1):
                s = slice(GC * j + 8 * o, GC * j + 8 * o + 8)
                t = slice(GC * (i - j) + 8 * o, GC * (i - j) + 8 * o + 8)
                pr = (r.kf[t, 0:T] * r.us[s, :], r.kd2[t, :] * r.uf[s, 0:T], r.kf[t, T:] * r.uf[s, T:])
                acc = pr if acc is None else tuple(a_ + p_ for a_, p_ in zip(acc, pr))
                yield 8, ('running', list(acc))
            acc = (acc[0] - acc[2], acc[0] + acc[1])
            s = slice(GC * i + 8 * o, GC * i + 8 * o + 8)
            r.yf[s, 0:T] = acc[0]
            r.yf[s, T:] = acc[1]
            yield 0, list(acc)
        if i % 4 == 0:
            r.pending.append(i // 4)


def _ssm_inverse(c0, r, q):
    rows = pl.ds(c0, GC)
    y = jnp.dot(r.yf[4 * GC * q:4 * GC * (q + 1), :].astype(BF16), r.inv[...],
                preferred_element_type=F32)
    skip = r.dskip[rows, :]
    for i in range(4):
        at = slice(T * (4 * q + i), T * (4 * q + i + 1))
        r.yt[rows, at] = y[GC * i:GC * i + GC] + skip * r.u[rows, at].astype(F32)


class _Refs:
    pass


def _kernel(ut_hbm, are_hbm, aim_hbm, bre_hbm, bim_hbm, cre_hbm, cim_hbm, ldt_hbm, dsk_hbm,
            xt_hbm, wq_hbm, wkt_hbm, wvt_hbm, wo_hbm, fwd_hbm, inv_hbm,
            out_hbm,
            u_v, are_v, aim_v, bre_v, bim_v, cre_v, cim_v, x_v, wq_v, wo_v, fwd_v, inv_v,
            ldt_ref, dsk_ref, wkt_ref, wvt_ref,
            wkv_s, wqt_s, wot_s, ke_s, ko_s, ve_s, vo_s, q_s, qo_s, sa_s, sb_s, ot_s, part_s, acc_s,
            dt_s, dskip_s, tab_l, tab_r, tab_s, edge_s, kd_s, uf_s, kf_s, yf_s, yt_s, us_s, ks_s,
            stage_a, stage_b, in_sem, out_sem):
    r = _Refs()
    r.mxu = []
    r.us, r.kd2 = us_s, ks_s
    r.u, r.a_re, r.a_im, r.b_re, r.b_im, r.c_re, r.c_im = u_v, are_v, aim_v, bre_v, bim_v, cre_v, cim_v
    r.fwd, r.inv, r.dt, r.dskip = fwd_v, inv_v, dt_s, dskip_s
    r.tab_l, r.tab_r, r.tab_s, r.edge, r.kd, r.uf, r.kf, r.yf, r.yt = (
        tab_l, tab_r, tab_s, edge_s, kd_s, uf_s, kf_s, yf_s, yt_s)

    sems = iter(range(in_sem.shape[0]))

    def load(src, dst, idx=None):
        if idx is not None:
            src, dst = src.at[idx], dst.at[idx]
        return pltpu.make_async_copy(src, dst, in_sem.at[next(sems)])

    ssm_in = [(are_hbm, are_v), (aim_hbm, aim_v), (bre_hbm, bre_v), (bim_hbm, bim_v),
              (cre_hbm, cre_v), (cim_hbm, cim_v), (ut_hbm, u_v)]
    ld_kv = [load(wkt_hbm, wkt_ref), load(wvt_hbm, wvt_ref)]
    ld_x = [load(xt_hbm, x_v, (slice(None), pl.ds(j * TQ, TQ))) for j in range(L // TQ)]
    ld_q = load(wq_hbm, wq_v)
    ld_small = [load(ldt_hbm, ldt_ref), load(dsk_hbm, dsk_ref)]
    ld_first = [load(s_, d_, pl.ds(384, D - 384)) for s_, d_ in ssm_in]
    ld_first += [load(fwd_hbm, fwd_v), load(inv_hbm, inv_v)]
    ld_rest = [load(s_, d_, pl.ds(0, 384)) for s_, d_ in ssm_in] + [load(wo_hbm, wo_v)]
    for cp in [ld_q] + ld_kv + ld_x[:3] + ld_small:
        cp.start()

    def column(ref):
        wide = jnp.concatenate([ref, jnp.zeros((1, 512 - D), F32)], axis=1)
        return jnp.broadcast_to(wide, (128, 512)).T[:D]

    def transposed(w):
        n = w.shape[1]
        w = jnp.concatenate([w.astype(F32), jnp.zeros((512 - D, n), F32)], axis=0)
        if n % 128:
            w = jnp.concatenate([w, jnp.zeros((512, -n % 128), F32)], axis=1)
        return w.T[:n, :D]

    tab_l[:, :, 8 * PITCH:16 * PITCH, :] = jnp.zeros((GC // 8, 4, 8 * PITCH, 128), F32)
    uf_s[...] = jnp.zeros(uf_s.shape, F32)
    kf_s[...] = jnp.zeros(kf_s.shape, F32)
    us_s[...] = jnp.zeros(us_s.shape, F32)
    ks_s[...] = jnp.zeros(ks_s.shape, F32)
    wkv_s[...] = jnp.zeros(wkv_s.shape, F32)
    acc_s[...] = jnp.ones(acc_s.shape, F32)
    for cp in ld_kv:
        cp.wait()
    wkv_s[0:DH, :] = wkt_ref[...].astype(F32)
    wkv_s[32:32 + DH, :] = wvt_ref[...].astype(F32)

    def project_kv(j):
        cols = slice(j * TQ, (j + 1) * TQ)
        kv = jnp.dot(wkv_s[...].astype(BF16), x_v[:, cols], preferred_element_type=F32)
        k_t = kv[0:32]
        v_t = jnp.where(lax.broadcasted_iota(jnp.int32, (32, TQ), 0) == DH, 1.0, kv[32:64])
        words = lambda v: pltpu.bitcast(v.astype(BF16), jnp.uint32)
        ve_s[:, cols] = words(v_t)
        vo_s[:, cols] = words(pltpu.roll(v_t, 4, 0))
        pad = jnp.zeros((96, TQ), F32)
        half = slice(j * TQ // 2, (j + 1) * TQ // 2)
        ke_s[half, :] = words(jnp.concatenate([k_t, pad], axis=0).T)
        ko_s[half, :] = words(jnp.concatenate([pltpu.roll(k_t, 4, 0), pad], axis=0).T)

    def project_q(j, lo=0, hi=D):
        cols = slice(j * TQ, (j + 1) * TQ)
        q_s[j % 2, lo:hi, :] = QSCALE * jnp.dot(wqt_s[lo:hi, :], x_v[:, cols], preferred_element_type=F32)

    def head_step(k_ref, q_t, dst, src, m_src, v_ref, side, state, chunks=range(L // CK), m_new=None):
        acc = None
        if src is not None:
            m_src = jnp.broadcast_to(jnp.max(m_src, axis=0, keepdims=True), (8, TQ))
        never = tab_l[0, 0, 15 * PITCH:15 * PITCH + 8, :] > 0.0
        for c in chunks:
            ks = slice(c * CK, (c + 1) * CK)

            def scores(lo, hi):
                if dst is None or lo == hi:
                    return m_new
                keys = pltpu.bitcast(k_ref[lo // 2:hi // 2, :], BF16)[:, 0:32]
                s = jnp.dot(keys, q_t, preferred_element_type=F32)
                dst[lo:hi, :] = s
                mc = jnp.max(s.reshape((hi - lo) // 8, 8, TQ), axis=0)
                return mc if m_new is None else jnp.maximum(m_new, mc)

            def numerators(tokens):
                m_c = [m_src[:, 128 * i:128 * i + 128] for i in range(TQ // 128)]
                m_hi = list(m_c)
                for i, tok in enumerate(tokens):
                    k = (i + state['knob']('turn', 0)) % len(m_c)
                    m_hi[k] = jnp.where(never, tok, m_hi[k])
                h = state['knob']('free', 120)
                parts = [src[c * CK + lo:c * CK + hi, :].reshape((hi - lo) // 8, 8, TQ)
                         - jnp.concatenate(mm, axis=1)
                         for lo, hi, mm in ((0, h, m_c), (h, CK, m_hi)) if hi > lo]
                return jnp.exp2(jnp.concatenate(parts, axis=0).reshape(CK, TQ)).astype(BF16)

            tokens = state['tokens'] if state else []
            side()
            todo = r.mxu[:state['knob']('matmuls', 1)] if state else []
            del r.mxu[:len(todo)]
            cut = c * CK + (state['knob']('cut', 80) if todo else CK)
            m_new = scores(c * CK, cut)
            for matmul in todo:
                matmul()
            m_new = scores(cut, (c + 1) * CK)
            if src is not None:
                p = numerators(tokens)
                o = jnp.dot(pltpu.bitcast(v_ref[:, ks], BF16), p, preferred_element_type=F32)
                acc = o if acc is None else acc + o
        return m_new, acc

    def finish_pair(base):
        acc_o = acc_s[0:32, :]
        o_o = acc_o * (1.0 / acc_o[0:1])
        mixed = jnp.where(
            lax.broadcasted_iota(jnp.int32, (8, TQ), 0) < 4, acc_s[32:40, :], o_o[0:8])
        ot_s[pl.ds(base + 24, 32), :] = jnp.concatenate([mixed, o_o[8:32]], axis=0)

    def iteration(it, m_even, with_ssm, last=False):
        def first_channel(g):
            if isinstance(g, int):
                return (g + NG - 4) % NG * GC
            return _aligned(jnp.where(g < 4, g + NG - 4, g - 4) * GC, GC)

        def knob(name, default):
            return PLACEMENT[name].get(state['step'], default) if with_ssm == 2 else default

        def spread(gen, total, steps):
            done = 0
            for step in range(1, steps + 1):
                tokens, latest = [], []
                while step == steps or done < total * (step + knob('shift', 0)) / steps:
                    cost, tok = next(gen, (None, []))
                    if cost is None:
                        break
                    if isinstance(tok, tuple):
                        latest = tok[1]
                    else:
                        tokens += tok
                    done += cost
                yield tokens + latest

        def ssm_work():
            prev = first_channel(it - 1 if isinstance(it, int) else jnp.maximum(it - 1, 0))
            r.pending = []
            late = []

            def drain():
                ready, r.pending[:] = list(r.pending), []
                for q in ready:
                    r.mxu.append(lambda q=q: _ssm_inverse(prev, r, q))
                    if with_ssm == 2:
                        r.mxu.append(lambda q=q: late.extend(r.transform(q)))

            if with_ssm == 2:
                yield from spread(_ssm_powers(first_channel(it), r),
                                  4 * (130 + 170), 8)
                yield from spread(_ssm_kernel_values(r), 8 * 228, 9)
                regroup = spread(_ssm_spectra(first_channel(it), r), 200, 2)
            products = spread(_ssm_products(r), 2 * 136 * 8, 12 if with_ssm == 2 else 28)
            for k in range(2 * L // CK):
                tokens = list(late)
                late[:] = []
                drain()
                tokens += next(products, [])
                if with_ssm == 2 and k in (1, 1 + 1):
                    tokens += next(regroup)
                yield tokens

        def early_projection():
            for c in range(L // CK):
                yield []
            EP = 64
            for lo in range(0, D, EP):
                part_s[lo:lo + EP, :] = jnp.dot(
                    wot_s[lo:lo + EP, 0:384], ot_s[0:384, :].astype(BF16), preferred_element_type=F32)
                for _ in range(EP // 32):
                    yield []

        def last_channels():
            for lo in range(0, L, 128):
                finish_channels(2, lo, lo + 128)
                yield []

        work = last_channels() if with_ssm == 4 else iter(()) if with_ssm == 3 else ssm_work() if with_ssm else early_projection()
        state = dict(tokens=[], step=-1, knob=knob)

        def side():
            state['step'] += 1
            state['tokens'] = next(work, [])

        base = _aligned((it & (NPAIR - 1)) * 2 * DH, 8)
        finish_pair(_aligned(((it + NPAIR - 1) & (NPAIR - 1)) * 2 * DH, 8))
        q_odd = pltpu.bitcast(qo_s[...], BF16)
        m_odd, acc_e = head_step(ko_s, q_odd, sb_s, sa_s, m_even, ve_s, side, state)
        o_e = acc_e * (1.0 / acc_e[DH:DH + 1])
        ot_s[pl.ds(base, 24), :] = o_e[0:24]
        acc_s[32:40, :] = o_e[24:32]
        if last:
            m_even, acc_o = head_step(None, None, None, sb_s, m_odd, vo_s, side, state)
        else:
            nxt = _aligned(((it + 1) & (NPAIR - 1)) * 2 * DH, 8)
            slot = ((it + 1) >> 3) & 1
            q_even = q_s[slot, pl.ds(nxt, 32), :].astype(BF16)
            qo_s[...] = pltpu.bitcast(q_s[slot, pl.ds(nxt + 24, 32), :].astype(BF16), jnp.uint32)
            m_even, acc_o = head_step(ke_s, q_even, sa_s, sb_s, m_odd, vo_s, side, state)
        for _ in work:
            pass
        for matmul in r.mxu:
            matmul()
        r.mxu[:] = []
        acc_s[0:32, :] = acc_o
        return m_even

    def b_copy(j):
        return pltpu.make_async_copy(
            stage_b.at[j], out_hbm.at[pl.ds(j * TQ, TQ), pl.ds(384, 512)], out_sem.at[j])

    def a_copy(c):
        return pltpu.make_async_copy(
            stage_a.at[c], out_hbm.at[:, pl.ds(128 * c, 128)], out_sem.at[4 + c])

    def finish_tile(j):
        cols = slice(j * TQ, (j + 1) * TQ)
        o = jnp.dot(wot_s[...], ot_s[...].astype(BF16), preferred_element_type=F32)
        z = jnp.concatenate([yt_s[384:D, cols], o], axis=0)
        stage_b[j] = z.T.astype(BF16)

    def finish_channels(c, lo=0, hi=L):
        stage_a[c, lo:hi, :] = yt_s[128 * c:128 * c + 128, lo:hi].T.astype(BF16)

    def first_scores(lo, hi, m):
        return head_step(ke_s, q_s[0, 0:32, :].astype(BF16), sa_s, None, None, None, lambda: None,
                         None, range(lo // CK, hi // CK), m)[0]

    ld_q.wait()
    wqt_s[...] = transposed(wq_v[...]).astype(BF16)
    ld_x[0].wait()
    for cp in ld_x[3:] + ld_first:
        cp.start()
    project_kv(0)
    project_q(0)
    qo_s[...] = pltpu.bitcast(q_s[0, 24:56, :].astype(BF16), jnp.uint32)
    ld_x[1].wait()
    for cp in ld_small:
        cp.wait()
    def columns():
        dt_s[...] = column(jnp.exp(ldt_ref[...].astype(F32).reshape(1, D)).astype(BF16).astype(F32))
        dskip_s[...] = column(dsk_ref[...].astype(F32).reshape(1, D))

    project_kv(1)
    project_q(1)
    columns()
    ld_x[2].wait()
    ld_x[3].wait()
    for cp in ld_rest:
        cp.start()
    project_kv(2)
    project_kv(3)
    m = first_scores(0, L, None)
    for cp in ld_first:
        cp.wait()

    def end_of_tile(j):
        finish_pair(D - 2 * DH)
        if j == 0:
            wot_s[...] = transposed(wo_v[...]).astype(BF16)
        if j < 2:
            project_q(j + 2)
        if j > 0:
            finish_channels(j - 1)
        finish_tile(j)
        b_copy(j).start()
        if j > 0:
            a_copy(j - 1).start()

    def main_body(it, m):
        m = iteration(it, m, 2)

        @pl.when((it & 3) == 3)
        def _():
            @pl.when(it == 3)
            def _():
                for cp in ld_rest:
                    cp.wait()

            for j in range(3):
                pl.when(it == (j + 1) * NPAIR - 1)(lambda j=j: end_of_tile(j))
        return m

    m = lax.fori_loop(0, NG, main_body, m)
    m = iteration(NG, m, 1)
    m = iteration(NG + 1, m, 4)
    a_copy(2).start()
    m = iteration(NG + 2, m, 3)
    b_copy(1).wait()
    iteration(NIT - 1, m, 0, last=True)
    j = L // TQ - 1
    last_copies = [pltpu.make_async_copy(
        stage_b.at[j, :, pl.ds(128 * i, 128)],
        out_hbm.at[pl.ds(j * TQ, TQ), pl.ds(384 + 128 * i, 128)], out_sem.at[j if i == 3 else 7 + i])
        for i in range(4)]
    finish_pair(D - 2 * DH)
    o_last = ot_s[384:D, :].astype(BF16)
    for i in range(4):
        lo, hi = max(128 * i - 64, 0), 128 * i + 64
        z = part_s[lo:hi, :] + jnp.dot(wot_s[lo:hi, 384:D], o_last, preferred_element_type=F32)
        if i == 0:
            z = jnp.concatenate([yt_s[384:D, j * TQ:], z], axis=0)
        stage_b[j, :, 128 * i:128 * i + 128] = z.T.astype(BF16)
        last_copies[i].start()
    b_copy(0).wait()
    b_copy(2).wait()
    for c in range(3):
        a_copy(c).wait()
    for cp in last_copies:
        cp.wait()


@jax.jit
def pallas_concat_heads__ssm_conv_s4__grouped_kv_mqa__prompt_kernel(
    A_u: jax.Array,
    A_A_re: jax.Array,
    A_A_im: jax.Array,
    A_B_re: jax.Array,
    A_B_im: jax.Array,
    A_C_re: jax.Array,
    A_C_im: jax.Array,
    A_log_dt: jax.Array,
    A_Dskip: jax.Array,
    B_x: jax.Array,
    B_wq: jax.Array,
    B_wk: jax.Array,
    B_wv: jax.Array,
    B_wo: jax.Array,
):
    hbm = pl.BlockSpec(memory_space=pl.ANY)
    scratch = [
        pltpu.VMEM((D, L), BF16),
        *[pltpu.VMEM((D, N), BF16) for _ in range(6)],
        pltpu.VMEM((D, L), BF16),
        pltpu.VMEM((D, D), BF16), pltpu.VMEM((D, D), BF16),
        pltpu.VMEM((5, T, 2 * T), BF16), pltpu.VMEM((2 * T, T), BF16),
        pltpu.VMEM((D,), BF16), pltpu.VMEM((D,), BF16),
        pltpu.VMEM((DH, D), BF16), pltpu.VMEM((DH, D), BF16),
        pltpu.VMEM((64, D), F32),
        pltpu.VMEM((D, D), BF16),
        pltpu.VMEM((D, D), BF16),
        pltpu.VMEM((L // 2, 128), jnp.uint32), pltpu.VMEM((L // 2, 128), jnp.uint32),
        pltpu.VMEM((16, L), jnp.uint32), pltpu.VMEM((16, L), jnp.uint32),
        pltpu.VMEM((2, D, TQ), F32), pltpu.VMEM((16, TQ), jnp.uint32),
        pltpu.VMEM((L, TQ), F32), pltpu.VMEM((L, TQ), F32),
        pltpu.VMEM((D, TQ), F32), pltpu.VMEM((D, TQ), F32), pltpu.VMEM((40, TQ), F32),
        pltpu.VMEM((D, 128), F32), pltpu.VMEM((D, 128), F32),
        pltpu.VMEM((GC // 8, 4, 16 * PITCH + 8, 128), F32),
        pltpu.VMEM((GC // 8, 4, 8 * PITCH + 8, 128), F32),
        pltpu.VMEM((GC // 8, 4, 8, 128), F32),
        pltpu.VMEM((GC // 8, 3, 8, 128), F32),
        pltpu.VMEM((8 * 17 + 16, 128), F32),
        pltpu.VMEM((NB * GC, 2 * T), F32), pltpu.VMEM((NB * GC, 2 * T), F32),
        pltpu.VMEM((NB * GC, 2 * T), F32),
        pltpu.VMEM((D, L), F32),
        pltpu.VMEM((NB * GC, T), F32), pltpu.VMEM((NB * GC, T), F32),
        pltpu.VMEM((3, L, 128), BF16), pltpu.VMEM((L // TQ, TQ, 512), BF16),
        pltpu.SemaphoreType.DMA((26,)), pltpu.SemaphoreType.DMA((10,)),
    ]
    out = pl.pallas_call(
        _kernel,
        out_shape=jax.ShapeDtypeStruct((L, 2 * D), BF16),
        in_specs=[hbm] * 16,
        out_specs=hbm,
        scratch_shapes=scratch,
        compiler_params=pltpu.CompilerParams(vmem_limit_bytes=100 * 1024 * 1024),
    )(A_u.reshape(L, D).T, A_A_re, A_A_im, A_B_re, A_B_im, A_C_re, A_C_im,
      A_log_dt, A_Dskip,
      B_x.reshape(L, D).T, B_wq, B_wk.T, B_wv.T, B_wo, _FWD_MATS, _INV_MAT)
    return out.reshape(1, L, 2 * D)
```
